```python
import os as _os
_os.environ.setdefault("JAX_PLATFORMS", "cpu")
import jax
import jax.numpy as jnp

def _softmax(x, axis=-1):
    return jax.nn.softmax(x, axis=axis)
def _gelu(x):
    return jax.nn.gelu(x, approximate=True)
def _silu(x):
    return jax.nn.silu(x)
def _sigmoid(x):
    return jax.nn.sigmoid(x)
def _layernorm(x, axis=-1, eps=1e-5):
    m = jnp.mean(x, axis=axis, keepdims=True)
    v = jnp.var(x, axis=axis, keepdims=True)
    return (x - m) / jnp.sqrt(v + eps)
def _scatter_add(tgt, idx, src, axis=0):
    return tgt.at[idx].add(src)
def _segment_sum(src, seg, n):
    return jax.ops.segment_sum(src, seg, n)
class _Rng:
    def __init__(self, key):
        self._k = key
    def _next(self):
        self._k, sub = jax.random.split(self._k)
        return sub
    def normal(self, shape):
        return jax.random.normal(self._next(), shape, dtype=jnp.bfloat16)
    def randint(self, lo, hi, shape):
        return jax.random.randint(self._next(), shape, lo, hi, dtype=jnp.int32)
    def uniform(self, shape, lo=0.0, hi=1.0):
        return jax.random.uniform(self._next(), shape, jnp.bfloat16, lo, hi)
    def permutation(self, n):
        return jax.random.permutation(self._next(), n)


kernel_name = 'concat_heads__ssm_conv_s4__linear_attn_block__prompt'

def setup_inputs():
    _rng = _Rng(jax.random.key(int.from_bytes(__import__("os").urandom(4), "little")))
    _w = (lambda a: (lambda t: t.astype(jnp.bfloat16) if jnp.issubdtype(t.dtype, jnp.floating) else t)(jnp.asarray(a)))
    def _A_setup():
        B, L, D, N = 1, 2048, 512, 128
        A_re = -jnp.exp((lambda *s: _rng.normal(s) * 0.1)(D, N))
        A_im = jnp.pi * (lambda *s: _rng.normal(s) * 0.1)(D, N)
        B_re = (lambda *s: _rng.normal(s) * 0.1)(D, N)
        B_im = (lambda *s: _rng.normal(s) * 0.1)(D, N)
        C_re = (lambda *s: _rng.normal(s) * 0.1)(D, N)
        C_im = (lambda *s: _rng.normal(s) * 0.1)(D, N)
        log_dt = (lambda *s: _rng.normal(s) * 0.1)(D) * 0.5 - 4.0
        Dskip = (lambda *s: _rng.normal(s) * 0.05)(D)
        return {
            "u": _w((lambda *s: _rng.normal(s) * 0.05)(B, L, D)),
            "A_re": _w(A_re),
            "A_im": _w(A_im),
            "B_re": _w(B_re),
            "B_im": _w(B_im),
            "C_re": _w(C_re),
            "C_im": _w(C_im),
            "log_dt": _w(log_dt),
            "Dskip": _w(Dskip),
        }
    _A_in = _A_setup()

    def _B_setup():
        B, S, D = 1, 2048, 512
        return {
            "x": _w((lambda *s: _rng.normal(s) * 0.05)(B, S, D)),
            "wqkv": _w((lambda *s: _rng.normal(s) * 0.4)(D, 3 * D)),
            "wo": _w((lambda *s: _rng.normal(s) * 0.05)(D, D)),
        }
    _B_in = _B_setup()

    return {
        "A_u": _A_in["u"],
        "A_A_re": _A_in["A_re"],
        "A_A_im": _A_in["A_im"],
        "A_B_re": _A_in["B_re"],
        "A_B_im": _A_in["B_im"],
        "A_C_re": _A_in["C_re"],
        "A_C_im": _A_in["C_im"],
        "A_log_dt": _A_in["log_dt"],
        "A_Dskip": _A_in["Dskip"],
        "B_x": _B_in["x"],
        "B_wqkv": _B_in["wqkv"],
        "B_wo": _B_in["wo"],
    }

def reference(A_u, A_A_re, A_A_im, A_B_re, A_B_im, A_C_re, A_C_im, A_log_dt, A_Dskip, B_x, B_wqkv, B_wo):
    def _A_ref(u, A_re, A_im, B_re, B_im, C_re, C_im, log_dt, Dskip):
        Bsz, L, D = u.shape
        dt = jnp.exp(log_dt)[:, None]
        A = A_re + 1j * A_im
        Bc = B_re + 1j * B_im
        Cc = C_re + 1j * C_im
        logdA = dt * A
        dB = dt * Bc
        l = (lambda x, dt: x.astype(dt))(jnp.arange(L), A_re.dtype)
        P = jnp.exp(logdA[:, :, None] * l[None, None, :])
        K = jnp.einsum("dn,dnl,dn->dl", Cc, P, dB).real
        L2 = 2 * L
        Kp = jnp.pad(K, ((0, 0), (0, L)))
        up = (lambda x, *d: x.transpose(*d))(u, 0, 2, 1)
        up = jnp.pad(up, ((0, 0), (0, 0), (0, L)))
        Kf = (lambda x, axes=(-2,-1): jnp.fft.rfft2(x.astype(jnp.float32), axes=axes))(Kp[:, None, :], axes=(-2, -1))
        Uf = (lambda x, axes=(-2,-1): jnp.fft.rfft2(x.astype(jnp.float32), axes=axes))(up[:, :, None, :], axes=(-2, -1))
        Yf = Uf * Kf[None, :, :, :]
        y = (lambda x, s, axes=(-2,-1): jnp.fft.irfft2(x, s=s, axes=axes).astype(jnp.bfloat16))(Yf, (1, L2), axes=(-2, -1))[:, :, 0, :L]
        y = (lambda x, *d: x.transpose(*d))(y, 0, 2, 1) + u * Dskip[None, None, :]
        return y

    def _B_ref(x, wqkv, wo):
        B, S, D = x.shape
        H = 32; Dh = D // H
        qkv = (lambda x, *d: x.transpose(*d))((x @ wqkv).reshape(B, S, 3, H, Dh), 2, 0, 3, 1, 4)
        q, k, v = qkv[0], qkv[1], qkv[2]
        phi = lambda t: jnp.where(t > 0, t + 1, jnp.exp(t)) + 1e-6
        pq, pk = phi(q), phi(k)
        kv = jnp.einsum("bhsd,bhse->bhde", pk, v)
        z = jnp.einsum("bhsd->bhd", pk)
        num = jnp.einsum("bhqd,bhde->bhqe", pq, kv)
        den = jnp.einsum("bhqd,bhd->bhq", pq, z)[..., None] + 1e-6
        o = num / den
        return (lambda x, *d: x.transpose(*d))(o, 0, 2, 1, 3).reshape(B, S, D) @ wo

    a = _A_ref(A_u, A_A_re, A_A_im, A_B_re, A_B_im, A_C_re, A_C_im, A_log_dt, A_Dskip)
    b = _B_ref(B_x, B_wqkv, B_wo)
    return jnp.concatenate([a, b], axis=-1)
```

```python
import numpy as np
import jax
import jax.numpy as jnp
from jax import lax
import jax.experimental.pallas as pl
import jax.experimental.pallas.tpu as pltpu
import ml_dtypes

F = jnp.float32
BF = jnp.bfloat16


def _consts():
    f1 = np.arange(32) + 0.5
    th = 2 * np.pi * f1[:, None] * np.arange(32)[None] / 64
    c = np.concatenate([np.cos(th), -np.sin(th)], 0)
    b1 = np.kron(np.eye(4), c)
    bi = np.kron(np.eye(2), c.reshape(2, 32, 32).transpose(2, 1, 0).reshape(32, 64))
    t = np.arange(64)
    ph = 2 * np.pi * (f1[:, None, None] * t[None, None] / 4096
                      + t[None, :, None] * t[None, None] / 64)
    co, si = np.cos(ph), np.sin(ph)
    m = np.concatenate([np.concatenate([co, si], 2),
                        np.concatenate([-si, co], 2)], 1)
    bf = ml_dtypes.bfloat16
    return b1.astype(bf), bi.astype(bf), m.astype(bf), m.transpose(0, 2, 1).astype(bf)


def _cm(a, b):
    return a[0] * b[0] - a[1] * b[1], a[0] * b[1] + a[1] * b[0]


def _dot(a, b):
    return jnp.dot(a, b, preferred_element_type=F)


def _kern(u_h, x_h, wq_h, wo_h, m_h, mi_h, ar, ai, br, bi, cr, ci, ldt, dsk, b1, b2,
          o_h, u, x, wq, wo, m, mi, oa, ob, pq, T, SK, SU, V, sem):
    cp = lambda s, d, i: pltpu.make_async_copy(s, d, sem.at[i])
    cps = [cp(u_h, u, 0), cp(x_h, x, 1), cp(wq_h, wq, 2), cp(wo_h, wo, 3),
           cp(m_h, m, 4), cp(mi_h, mi, 5)]
    for c in cps[1:3] + cps[:1] + cps[3:]:
        c.start()
    lane = lax.broadcasted_iota(jnp.int32, (8, 128), 1)

    def grp(g, _):
        r = pl.ds(pl.multiple_of(g * 16, 16), 16)
        ld = lambda f: f[r, :].astype(F)
        dt = jnp.exp(ld(ldt)).astype(BF).astype(F)
        e = jnp.exp(dt * ld(ar))
        p = dt * ld(ai)
        z = (e * jnp.cos(p), e * jnp.sin(p))
        w = _cm((ld(cr), ld(ci)), (dt * ld(br), dt * ld(bi)))
        P = [(jnp.ones_like(e), jnp.zeros_like(e)), z]
        for s in range(2, 16):
            P.append(_cm(P[s // 2], P[s - s // 2]))
        Es, Gs = [], []
        cur = w
        for n in (16, 8, 8, 9):
            Es.append(P)
            st = _cm(P[8], P[8])
            G = []
            for j in range(n):
                G.append(cur)
                if not (n == 9 and j == 8):
                    cur = _cm(cur, st)
            Gs.append(G)
            P = P[::2] + [_cm(q, q) for q in P[8:]]
        c2 = lambda q, sg: jnp.concatenate([q[0], sg * q[1]], 1)
        for h in range(2):
            hs = slice(8 * h, 8 * h + 8)
            rows = []
            for E, G in zip(Es, Gs):
                Em = jnp.concatenate([c2(q, 1.0)[hs] for q in E], 0).astype(BF)
                Gm = jnp.concatenate([c2(q, -1.0)[hs] for q in G], 0).astype(BF)
                R = lax.dot_general(Gm, Em, (((1,), (1,)), ((), ())),
                                    preferred_element_type=F)
                R = R.reshape(len(G), 8, 128)
                sub = lax.broadcasted_iota(jnp.int32, (1, 8, 128), 1)
                rows.append(jnp.sum(jnp.where(sub == (lane & 7)[None], R, 0.0), axis=1))
            rows.append(jnp.zeros((7, 128), F))
            V[2 * g + h] = jnp.concatenate(rows, 0)
        return 0
    cps[1].wait()
    cps[2].wait()
    rb = lambda t: t.astype(BF).astype(F)
    phi = lambda t: rb(jnp.where(t > 0, rb(t + 1), rb(jnp.exp(t))) + 1e-6).astype(BF)
    TM = 256
    kv = [jnp.zeros((128, 256), F)] * 4
    ones = jnp.ones((TM, 128), BF)
    def outer(i, kv):
        kv = list(kv)
        for k in range(4):
            grp(4 * i + k, 0)
        r = pl.ds(pl.multiple_of(i * TM, TM), TM)
        xx = x[r, :]
        pq[r, :] = phi(rb(_dot(xx, wq[:, 0:512])))
        pk = phi(rb(_dot(xx, wq[:, 512:1024])))
        v = _dot(xx, wq[:, 1024:1536]).astype(BF)
        for q in range(4):
            c = slice(q * 128, (q + 1) * 128)
            kv[q] = kv[q] + lax.dot_general(
                pk[:, c], jnp.concatenate([v[:, c], ones], 1),
                (((0,), (0,)), ((), ())), preferred_element_type=F)
        return tuple(kv)
    kv = lax.fori_loop(0, 8, outer, tuple(kv))
    TM = 512

    def trn(i, _):
        tl = i // 6
        jb = i % 6
        v = [V[tl * 16 + k, pl.ds(pl.multiple_of(jb * 8, 8), 8), :] for k in range(16)]
        for b in (1, 2, 4, 8):
            hi = (lane & (8 * b)) != 0
            n = list(v)
            for k in range(16):
                if not k & b:
                    n[k] = jnp.where(hi, pltpu.roll(v[k + b], 8 * b, 1), v[k])
                    n[k + b] = jnp.where(hi, v[k + b], pltpu.roll(v[k], 128 - 8 * b, 1))
            v = n
        for s in range(16):
            SU[tl, pl.ds(jb * 128 + s, 8, stride=16), :] = v[s]
        return 0
    lax.fori_loop(0, 24, trn, 0, unroll=2)
    for q in range(4):
        T[q, 0:256, :] = SU[q, 0:256, :]
        for base, src, per, tab in ((256, 256, 4, (0, 0, 1, 2)),
                                    (512, 384, 8, (0, 0, 0, 1, 1, 1, 2, 2)),
                                    (1024, 512, 16, (0,) * 5 + (1,) * 7 + (2,) * 4)):
            for r_, o in enumerate(tab):
                T[q, pl.ds(base + r_, 64, stride=per), :] = SU[q, pl.ds(src + o, 64, stride=2), :]

    def stage1(S):
        def b(i, _):
            for q in range(4):
                xx = jnp.concatenate(
                    [T[q, pl.ds(4 * i + k, 32, stride=64), :] for k in range(4)], 0)
                y = _dot(b1[...], xx.astype(BF))
                for k in range(4):
                    for ri in range(2):
                        o = k * 64 + ri * 32
                        S[q, pl.ds(4 * i + k + ri * 64, 32, stride=128), :] = y[o:o + 32]
            return 0
        lax.fori_loop(0, 16, b, 0, unroll=4)

    stage1(SK)
    cps[0].wait()
    for q in range(4):
        T[q] = u[:, q * 128:(q + 1) * 128].astype(F)
    stage1(SU)
    cps[4].wait()
    cps[5].wait()

    def s2(f, _):
        r = pl.ds(pl.multiple_of(f * 128, 128), 128)
        cat = lambda S: jnp.concatenate([S[q, r, :] for q in range(4)], 1).astype(BF)
        k = _dot(m[f], cat(SK))
        a = _dot(m[f], cat(SU))
        pr, pi = _cm((k[:64], k[64:]), (a[:64], a[64:]))
        z = _dot(mi[f], jnp.concatenate([pr, pi], 0).astype(BF))
        for q in range(4):
            SU[q, r, :] = z[:, q * 128:(q + 1) * 128]
        return 0
    lax.fori_loop(0, 32, s2, 0, unroll=4)

    def s3(i, _):
        for q in range(4):
            zz = jnp.concatenate([SU[q, pl.ds(2 * i + k, 64, stride=64), :]
                                  for k in range(2)], 0)
            y = _dot(b2[...], zz.astype(BF))
            for k in range(2):
                T[q, pl.ds(2 * i + k, 32, stride=64), :] = y[32 * k:32 * k + 32]
        return 0
    lax.fori_loop(0, 32, s3, 0, unroll=8)
    for q in range(4):
        c = slice(q * 128, (q + 1) * 128)
        y = (T[q] * (2.0 / 4096)).astype(BF).astype(F)
        sk = (u[:, c].astype(F) * dsk[:, c].astype(F)).astype(BF).astype(F)
        oa[:, c] = (y + sk).astype(BF)
    ca = cp(oa, o_h.at[:, 0:512], 6)
    ca.start()

    i0 = lax.broadcasted_iota(jnp.int32, (128, 256), 0) // 16
    i1 = (lax.broadcasted_iota(jnp.int32, (128, 256), 1) % 128) // 16
    kv = [jnp.where(i0 == i1, a, 0.0).astype(BF) for a in kv]
    cps[3].wait()
    for i in range(2048 // TM):
        r = slice(i * TM, (i + 1) * TM)
        os_ = []
        for q in range(4):
            nd = _dot(pq[r, q * 128:(q + 1) * 128], kv[q])
            os_.append((rb(nd[:, :128]) / rb(rb(nd[:, 128:]) + 1e-6)).astype(BF))
        ob[r, :] = _dot(jnp.concatenate(os_, 1), wo[...]).astype(BF)
    cb = cp(ob, o_h.at[:, 512:1024], 7)
    cb.start()
    ca.wait()
    cb.wait()


@jax.jit
def pallas_concat_heads__ssm_conv_s4__linear_attn_block__prompt_kernel(
    A_u, A_A_re, A_A_im, A_B_re, A_B_im, A_C_re, A_C_im, A_log_dt, A_Dskip,
    B_x, B_wqkv, B_wo,
):
    b1, b2, m, mi = _consts()
    H = pl.BlockSpec(memory_space=pl.ANY)
    Vm = pl.BlockSpec(memory_space=pltpu.VMEM)
    S = pltpu.VMEM
    out = pl.pallas_call(
        _kern,
        out_shape=jax.ShapeDtypeStruct((2048, 1024), BF),
        in_specs=[H] * 6 + [Vm] * 10,
        out_specs=H,
        scratch_shapes=[S((2048, 512), BF), S((2048, 512), BF), S((512, 1536), BF),
                        S((512, 512), BF), S((32, 128, 128), BF), S((32, 128, 128), BF),
                        S((2048, 512), BF), S((2048, 512), BF), S((2048, 512), BF),
                        S((4, 2048, 128), F), S((4, 4096, 128), F), S((4, 4096, 128), F),
                        S((64, 48, 128), F), pltpu.SemaphoreType.DMA((8,))],
        compiler_params=pltpu.CompilerParams(vmem_limit_bytes=100 * 2**20),
    )(A_u[0], B_x[0], B_wqkv, B_wo, m, mi, A_A_re, A_A_im, A_B_re, A_B_im, A_C_re,
      A_C_im, A_log_dt[:, None], A_Dskip[None], b1, b2)
    return out[None]
```
